```python
import jax
import jax.numpy as jnp

def _softmax(x, axis=-1):
    return jax.nn.softmax(x, axis=axis)
def _gelu(x):
    return jax.nn.gelu(x, approximate=True)
def _silu(x):
    return jax.nn.silu(x)
def _sigmoid(x):
    return jax.nn.sigmoid(x)
def _layernorm(x, axis=-1, eps=1e-5):
    m = jnp.mean(x, axis=axis, keepdims=True)
    v = jnp.var(x, axis=axis, keepdims=True)
    return (x - m) / jnp.sqrt(v + eps)
def _scatter_add(tgt, idx, src, axis=0):
    return tgt.at[idx].add(src)
def _segment_sum(src, seg, n):
    return jax.ops.segment_sum(src, seg, n)
class _Rng:
    def __init__(self, key):
        self._k = key
    def _next(self):
        self._k, sub = jax.random.split(self._k)
        return sub
    def normal(self, shape):
        return jax.random.normal(self._next(), shape, dtype=jnp.bfloat16)
    def randint(self, lo, hi, shape):
        return jax.random.randint(self._next(), shape, lo, hi, dtype=jnp.int32)
    def uniform(self, shape, lo=0.0, hi=1.0):
        return jax.random.uniform(self._next(), shape, jnp.bfloat16, lo, hi)
    def permutation(self, n):
        return jax.random.permutation(self._next(), n)


kernel_name = 'recurrent_scan__linear_kernel_hedgehog__dense_activation_relu__prompt'

def _fwd_setup_inputs():
    _rng = _Rng(jax.random.key(int.from_bytes(__import__("os").urandom(4), "little")))
    _w = (lambda a: (lambda t: t.astype(jnp.bfloat16) if jnp.issubdtype(t.dtype, jnp.floating) else t)(jnp.asarray(a)))
    def _A_setup():
        B, S, D, H = 1, 2048, 1024, 32
        Dh = D // H
        return {
            "x": _w((lambda *s: _rng.normal(s) * 0.05)(B, S, D)),
            "wqkv": _w((lambda *s: _rng.normal(s) * 0.05)(D, 3 * D)),
            "w_phi": _w((lambda *s: _rng.normal(s) * 0.05)(H, Dh, Dh) * (Dh ** -0.5)),
            "wo": _w((lambda *s: _rng.normal(s) * 0.05)(D, D)),
        }
    _A_in = _A_setup()

    def _B_setup():
        B, S, D, Dff = 1, 2048, 1024, 3584
        return {
            "x": _w((lambda *s: _rng.normal(s) * 0.05)(B, S, D)),
            "w1": _w((lambda *s: _rng.normal(s) * 0.05)(D, Dff)),
            "w2": _w((lambda *s: _rng.normal(s) * 0.05)(Dff, D)),
        }
    _B_in = _B_setup()

    return {
        "A_x": _A_in["x"],
        "A_wqkv": _A_in["wqkv"],
        "A_w_phi": _A_in["w_phi"],
        "A_wo": _A_in["wo"],
        "B_x": _B_in["x"],
        "B_w1": _B_in["w1"],
        "B_w2": _B_in["w2"],
    }

def _fwd_reference(A_x, A_wqkv, A_w_phi, A_wo, B_x, B_w1, B_w2):
    def _A_ref(x, wqkv, w_phi, wo):
        B, S, D = x.shape
        H = 32; Dh = D // H
        qkv = (lambda x, *d: x.transpose(*d))((x @ wqkv).reshape(B, S, 3, H, Dh), 2, 0, 3, 1, 4)
        q, k, v = qkv[0], qkv[1], qkv[2]
        pq = jnp.einsum("bhsd,hdf->bhsf", q, w_phi)
        pk = jnp.einsum("bhsd,hdf->bhsf", k, w_phi)
        phi_q = jnp.concatenate([_softmax(pq, axis=-1), _softmax(-pq, axis=-1)], axis=-1)
        phi_k = jnp.concatenate([_softmax(pk, axis=-1), _softmax(-pk, axis=-1)], axis=-1)
        kv = jnp.einsum("bhsf,bhsd->bhfd", phi_k, v)
        z  = jnp.einsum("bhsf->bhf", phi_k)
        num = jnp.einsum("bhqf,bhfd->bhqd", phi_q, kv)
        den = jnp.einsum("bhqf,bhf->bhq", phi_q, z)[..., None] + 1e-6
        o = num / den
        return (lambda x, *d: x.transpose(*d))(o, 0, 2, 1, 3).reshape(B, S, D) @ wo

    def _B_ref(x, w1, w2):
        h = jnp.einsum("bsd,df->bsf", x, w1)
        zero = jnp.zeros_like(h)
        h = jnp.maximum(h, zero)
        return jnp.einsum("bsf,fd->bsd", h, w2)

    x = A_x
    xn = _layernorm(x, axis=-1)
    s = _A_ref(xn, A_wqkv, A_w_phi, A_wo)
    g = _silu(_B_ref(xn, B_w1, B_w2))
    return x + s * g


def setup_inputs():
    _inp = _fwd_setup_inputs()
    _gk = jax.random.fold_in(jax.random.key(int.from_bytes(__import__("os").urandom(4), "little")), 2**31 - 1)
    _shapes = [[1, 2048, 1024]]
    _dtypes = ['bfloat16']
    _gks = jax.random.split(_gk, len(_shapes))
    _gs = [jax.random.normal(k, s, dtype=jnp.dtype(d)) * 0.05 for k, s, d in zip(_gks, _shapes, _dtypes)]
    _inp["grad_out"] = _gs[0]
    return _inp

def reference(A_x, A_wqkv, A_w_phi, A_wo, B_w1, B_w2, B_x, grad_out):
    _const = dict(B_x=B_x)
    def _f(*_d):
        return _fwd_reference(**{'A_x': _d[0], 'A_wqkv': _d[1], 'A_w_phi': _d[2], 'A_wo': _d[3], 'B_w1': _d[4], 'B_w2': _d[5], **_const})
    _out, _vjp = jax.vjp(_f, A_x, A_wqkv, A_w_phi, A_wo, B_w1, B_w2)
    _grads = _vjp(grad_out)
    _out0 = jnp.asarray(_out)
    return (_out0, *[jnp.asarray(_g) for _g in _grads])
```

```python
import jax
import jax.numpy as jnp
from jax import lax
import jax.experimental.pallas as pl
import jax.experimental.pallas.tpu as pltpu

S, D, H, DH, FF = 2048, 1024, 32, 32, 3584
TS = 256
NT = S // TS
TF = 256
NF = FF // TF
HC = 512
NHC = FF // HC
NP = H // 2
AUG = 80
F32 = jnp.float32
BF16 = jnp.bfloat16

_NN = (((1,), (0,)), ((), ()))
_NT = (((1,), (1,)), ((), ()))
_TN = (((0,), (0,)), ((), ()))
_TT = (((0,), (1,)), ((), ()))


def _mm(a, b, dn):
    return lax.dot_general(a, b, dn, preferred_element_type=F32)


def _rcp(x):
    r = pl.reciprocal(x, approx=True)
    return r * (2.0 - x * r)


def _softmax_pm(p):
    r, ts = p.shape
    nh = r // DH
    p3 = p.reshape(nh, DH, ts)
    mx = jnp.max(p3, axis=1, keepdims=True)
    mn = jnp.min(p3, axis=1, keepdims=True)
    ep = jnp.exp(p3 - mx)
    en = jnp.exp(mn - p3)
    ap = ep * _rcp(jnp.sum(ep, axis=1, keepdims=True))
    an = en * _rcp(jnp.sum(en, axis=1, keepdims=True))
    return jnp.concatenate([ap, an], axis=1).reshape(nh * 2 * DH, ts)


def _softmax_pm_bwd(phi, dphi):
    r, ts = phi.shape
    nh = r // (2 * DH)
    ph = phi.reshape(nh * 2, DH, ts)
    t = ph * dphi.reshape(nh * 2, DH, ts)
    dp = t - ph * jnp.sum(t, axis=1, keepdims=True)
    dp = dp.reshape(nh, 2 * DH, ts)
    return (dp[:, :DH, :] - dp[:, DH:, :]).reshape(nh * DH, ts)


def _rows(t):
    if isinstance(t, int):
        return pl.ds(t * TS, TS)
    return pl.ds(pl.multiple_of(t * TS, TS), TS)


def _kernel(x_hbm, wqkv_hbm, wphi_hbm, wo_hbm, w1_hbm, w2_hbm, dout_hbm,
            out_hbm, gx_hbm, dwqkv_hbm, dwphi_hbm, dwo_hbm, dw1_hbm, dw2_hbm,
            X, DO, WALL, WQK, WPHI, BD, WO, W1, W2, XN, RSTD, PHIK, DQKV, R,
            DB, DS, OT, DXN, KVZ, DKVZ, DKVZB, PHIQ, DND, DHF, DWP, GG, EE, PACC, FLAG,
            xsem, isem, osem):
    in_copies = []

    def cin(src, dst):
        c = pltpu.make_async_copy(src, dst, isem.at[len(in_copies)])
        c.start()
        in_copies.append(c)
        return c

    def x_copy(t):
        return pltpu.make_async_copy(x_hbm.at[_rows(t)], X.at[_rows(t)], xsem.at[t])

    def wrows(col, i, dst):
        return cin(wqkv_hbm.at[pl.ds(512 * i, 512), pl.ds(col, D)], dst.at[pl.ds(512 * i, 512), pl.ds(col, D)])

    FLAG[0] = 0
    x_copy(0).start()
    c_wv0 = wrows(2 * D, 0, WALL)
    c_wphi = cin(wphi_hbm, WPHI)

    out_copies = []

    def cout(src, dst):
        c = pltpu.make_async_copy(src, dst, osem.at[len(out_copies)])
        c.start()
        out_copies.append(c)

    def bdmask():
        row = lax.broadcasted_iota(jnp.int32, (128, 128), 0)
        col = lax.broadcasted_iota(jnp.int32, (128, 128), 1)
        return (row // DH) == (col // DH)

    def emat():
        e_r = lax.broadcasted_iota(jnp.int32, (DH, 128), 0)
        e_c = lax.broadcasted_iota(jnp.int32, (DH, 128), 1)
        return jnp.where((e_c % DH) == e_r, 1.0, 0.0).astype(BF16)

    def m80():
        r80 = lax.broadcasted_iota(jnp.int32, (AUG, 128), 0)
        c80 = lax.broadcasted_iota(jnp.int32, (AUG, 128), 1)
        return jnp.where(r80 < 64, r80 // DH, (r80 - 64) // 8) == (c80 // 64)

    def ln_tile(t):
        rows = _rows(t)
        x = X[rows, :].astype(F32)
        mu = jnp.mean(x, axis=1, keepdims=True)
        xc = x - mu
        var = jnp.mean(xc * xc, axis=1, keepdims=True)
        rstd = lax.rsqrt(var + 1e-5)
        xn = (xc * rstd).astype(BF16)
        XN[rows, :] = xn
        RSTD[rows, :] = jnp.broadcast_to(rstd, (TS, 128))
        return xn

    def fold(g, off, rs=slice(None)):
        sl = pl.ds(off + g * 128, 128)
        WALL[rs, sl] = _mm(WQK[rs, sl], BD[g], _NN).astype(BF16)

    def phik_tile(t, pk):
        rows = _rows(t)
        for c in range(8):
            PHIK[pl.ds(c * 256, 256), rows] = _softmax_pm(pk[c * 128:(c + 1) * 128]).astype(BF16)

    x_copy(0).wait()
    c_wv1 = wrows(2 * D, 1, WALL)
    c_wk0 = wrows(D, 0, WQK)
    xn0 = ln_tile(0)
    c_wv0.wait()
    c_wk1 = wrows(D, 1, WQK)
    x_copy(1).start()
    DXN[pl.ds(0, D), pl.ds(0, TS)] = _mm(WALL[pl.ds(0, 512), pl.ds(2 * D, D)], xn0[:, 0:512], _TT)
    c_wv1.wait()
    x_copy(2).start()
    x_copy(3).start()
    vt0 = DXN[pl.ds(0, D), pl.ds(0, TS)] + _mm(WALL[pl.ds(512, 512), pl.ds(2 * D, D)], xn0[:, 512:D], _TT)
    DQKV[pl.ds(2 * D, D), _rows(0)] = vt0.astype(BF16)
    c_wphi.wait()
    for g in range(8):
        wrep = _mm(WPHI[pl.ds(g * 128, 128), :], emat(), _NN)
        BD[g] = jnp.where(bdmask(), wrep, 0.0).astype(BF16)
    c_wk0.wait()
    for t in range(4, NT):
        x_copy(t).start()
    for g in range(8):
        fold(g, D, pl.ds(0, 512))
    c_wk1.wait()
    c_wq = cin(wqkv_hbm.at[:, pl.ds(0, D)], WQK.at[:, pl.ds(0, D)])
    c_w1 = cin(w1_hbm, W1)
    c_w2 = cin(w2_hbm, W2)
    c_do = cin(dout_hbm, DO)
    c_wo = cin(wo_hbm, WO)
    for g in range(8):
        fold(g, D, pl.ds(512, 512))

    def p1_body(t, xn):
        x_copy(t + 1).wait()
        pk = _mm(WALL[:, pl.ds(D, D)], xn, _TT)
        xn_next = ln_tile(t + 1)
        vt = _mm(WALL[:, pl.ds(2 * D, D)], xn_next, _TT)
        phik_tile(t, pk)
        DQKV[pl.ds(2 * D, D), _rows(t + 1)] = vt.astype(BF16)
        return xn_next

    xn_last = lax.fori_loop(0, NT - 1, p1_body, xn0)
    c_wq.wait()
    pk = _mm(WALL[:, pl.ds(D, D)], xn_last, _TT)
    for g in range(8):
        fold(g, 0)
    phik_tile(NT - 1, pk)

    c_w1.wait()

    def p1h_body(j, carry):
        fs = pl.ds(pl.multiple_of(j * HC, 128), HC)
        h = _mm(XN[...], W1[:, fs], _NN)
        R[:, fs] = jnp.where(h > 0.0, h, jnp.where(h == 0.0, 0.0, -0.0)).astype(BF16)
        return carry

    lax.fori_loop(0, NHC, p1h_body, 0)

    def ffn_b(t, c):
        cs = pl.ds(c * 256 if isinstance(c, int) else pl.multiple_of(c * 256, 256), 256)
        rows = _rows(t)
        b = _mm(R[rows, :], W2[:, cs], _NN)
        sig = 0.5 * jnp.tanh(0.5 * b) + 0.5
        g = b * sig
        dout = DO[rows, cs].astype(F32)
        DS[rows, cs] = (dout * g).astype(BF16)
        GG[t % 2, :, cs] = g
        EE[t % 2, :, cs] = dout * (sig + g * (1.0 - sig))

    ones_s = jnp.ones((16, S), BF16)
    for p in range(NP):
        v1 = jnp.concatenate([DQKV[pl.ds(2 * D + 64 * p, 64), :], ones_s], axis=0)
        kvz = _mm(v1, PHIK[pl.ds(128 * p, 128), :], _NT)
        KVZ[p] = jnp.where(m80(), kvz, 0.0).astype(BF16)
        DKVZ[p] = jnp.zeros((AUG, 128), F32)

    c_w2.wait()
    c_do.wait()

    def b0_body(c, carry):
        ffn_b(0, c)
        return carry

    lax.fori_loop(0, 4, b0_body, 0)
    c_wo.wait()

    def p2_tile(t, with_ffn):
        rows = _rows(t)
        ds = DS[rows, :]
        g = GG[t % 2]
        e = EE[t % 2]
        DXN[rows, :] = jnp.zeros((TS, D), F32)
        if with_ffn:
            ffn_b(t + 1, 0)
        pq = _mm(WALL[:, pl.ds(0, D)], XN[rows, :], _TT)
        dot_ = _mm(WO[...], ds, _NT)
        for c in range(8):
            PHIQ[pl.ds(c * 256, 256), :] = _softmax_pm(pq[c * 128:(c + 1) * 128]).astype(BF16)
        nds = [_mm(KVZ[p], PHIQ[pl.ds(128 * p, 128), :], _NN) for p in range(NP)]
        if with_ffn:
            ffn_b(t + 1, 1)
        for p in range(NP):
            nd = nds[p]
            rden = _rcp(nd[64:AUG].reshape(2, 1, 8, TS) + 1e-6)
            o4 = nd[0:64].reshape(2, 4, 8, TS) * rden
            OT[pl.ds(64 * p, 64), rows] = o4.reshape(64, TS).astype(BF16)
            dnum = dot_[64 * p:64 * (p + 1)].reshape(2, 4, 8, TS) * rden
            dden = -jnp.sum(dnum * o4, axis=1, keepdims=True)
            DND[p, pl.ds(0, 64), :] = dnum.reshape(64, TS).astype(BF16)
            DND[p, pl.ds(64, 16), :] = dden.reshape(16, TS).astype(BF16)
        dphis = []
        for p in range(NP):
            dnd = DND[p]
            dphis.append(_mm(KVZ[p], dnd, _TN))
            DKVZ[p] += _mm(dnd, PHIQ[pl.ds(128 * p, 128), :], _NT)
        s = _mm(OT[:, rows], WO[...], _TN)
        for p in range(NP):
            phi = PHIQ[pl.ds(128 * p, 128), :].astype(F32)
            DQKV[pl.ds(64 * p, 64), rows] = _softmax_pm_bwd(phi, dphis[p]).astype(BF16)
        if with_ffn:
            ffn_b(t + 1, 2)
            ffn_b(t + 1, 3)
        X[rows, :] = (X[rows, :].astype(F32) + s * g).astype(BF16)
        DB[rows, :] = (e * s).astype(BF16)

    def p2_body(t, carry):
        p2_tile(t, True)
        return carry

    lax.fori_loop(0, NT - 1, p2_body, 0)
    p2_tile(NT - 1, False)
    cout(X, out_hbm)

    for p in range(NP):
        DKVZB[p] = jnp.where(m80(), DKVZ[p], 0.0).astype(BF16)

    def kside(p):
        if isinstance(p, int):
            vs, ks, fs_ = pl.ds(2 * D + 64 * p, 64), pl.ds(D + 64 * p, 64), pl.ds(128 * p, 128)
        else:
            vs = pl.ds(pl.multiple_of(2 * D + 64 * p, 64), 64)
            ks = pl.ds(pl.multiple_of(D + 64 * p, 64), 64)
            fs_ = pl.ds(pl.multiple_of(128 * p, 128), 128)
        v1 = jnp.concatenate([DQKV[vs, :], ones_s], axis=0)
        dk = DKVZB[p]
        phi = PHIK[fs_, :]
        dphi = _mm(dk, v1, _TN)
        DQKV[vs, :] = _mm(dk[0:64], phi, _NN).astype(BF16)
        DQKV[ks, :] = _softmax_pm_bwd(phi.astype(F32), dphi).astype(BF16)

    for p in range(NF, NP):
        kside(p)

    base3 = len(out_copies)

    def dw_copies(j):
        fs = pl.ds(j * TF if isinstance(j, int) else pl.multiple_of(j * TF, 128), TF)
        return (pltpu.make_async_copy(W2.at[fs, :], dw2_hbm.at[fs, :], osem.at[base3 + 2 * j]),
                pltpu.make_async_copy(W1.at[:, fs], dw1_hbm.at[:, fs], osem.at[base3 + 2 * j + 1]))

    def p3_body(j, carry):
        fs = pl.ds(pl.multiple_of(j * TF, 128), TF)
        c2, c1 = dw_copies(j)
        dr = _mm(DB[...], W2[fs, :], _NT)
        r = R[:, fs].astype(F32)
        rb = lax.bitcast_convert_type(r, jnp.int32)
        DHF[...] = jnp.where(r > 0.0, dr, jnp.where(rb == 0, 0.5 * dr, 0.0)).astype(BF16)
        kside(j)
        W2[fs, :] = _mm(R[:, fs], DB[...], _TN).astype(BF16)
        c2.start()
        DXN[...] += _mm(DHF[...], W1[:, fs], _NT)
        W1[:, fs] = _mm(XN[...], DHF[...], _TN).astype(BF16)
        c1.start()
        return carry

    lax.fori_loop(0, NF, p3_body, 0)
    for j in range(NF):
        out_copies.extend(dw_copies(j))

    def dwo_chunk(c):
        cs = pl.ds(c * 128 if isinstance(c, int) else pl.multiple_of(c * 128, 128), 128)
        WO[:, cs] = _mm(OT[...], DS[:, cs], _NN).astype(BF16)

    def gx_tile(t, m1, m2):
        rows = _rows(t)
        xn = XN[rows, :].astype(F32)
        rstd = RSTD[rows, :][:, 0:1]
        return DO[rows, :].astype(F32) + rstd * (DXN[rows, :] - m1 - xn * m2)

    out_copies.pop(0).wait()

    def p4_body(t, carry):
        never = FLAG[0] != 0
        rows = _rows(t)
        tp = jnp.maximum(t - 1, 0)
        dwo_chunk(t)
        dxn = _mm(DQKV[:, rows], WALL[...], _TT) + DXN[rows, :]
        X[_rows(tp), :] = jnp.where(never, dxn, gx_tile(tp, *carry)).astype(BF16)
        m1 = jnp.mean(dxn, axis=1, keepdims=True)
        m2 = jnp.mean(dxn * XN[rows, :].astype(F32), axis=1, keepdims=True)
        DXN[rows, :] = dxn
        return m1, m2

    zc = jnp.zeros((TS, 1), F32)
    m12 = lax.fori_loop(0, NT, p4_body, (zc, zc))
    nsem = [len(out_copies) + 1]

    def cout2(src_, dst_):
        c = pltpu.make_async_copy(src_, dst_, osem.at[nsem[0]])
        nsem[0] += 1
        c.start()
        out_copies.append(c)

    cout2(WO, dwo_hbm)

    X[_rows(NT - 1), :] = gx_tile(NT - 1, *m12).astype(BF16)
    cout2(X, gx_hbm)
    for cidx in (4, 5):
        cs = pl.ds(cidx * 512, 512)
        WALL[:, cs] = _mm(XN[...], DQKV[cs, :], _TT).astype(BF16)
        cout2(WALL.at[:, cs], dwqkv_hbm.at[:, cs])

    for g in range(8):
        PACC[g] = jnp.zeros((128, 128), F32)
    base5 = nsem[0]
    nsem[0] += 4

    def g_copy(c):
        cs = pl.ds(c * 512 if isinstance(c, int) else pl.multiple_of(c * 512, 512), 512)
        return pltpu.make_async_copy(WALL.at[:, cs], dwqkv_hbm.at[:, cs], osem.at[base5 + c])

    def p5_body(c, carry):
        cs = pl.ds(pl.multiple_of(c * 512, 512), 512)
        gb = _mm(XN[...], DQKV[cs, :], _TT).astype(BF16)
        for gg in range(4):
            g = (c * 4 + gg) % 8
            gsl = gb[:, gg * 128:(gg + 1) * 128]
            sl = pl.ds(pl.multiple_of(c * 512 + gg * 128, 128), 128)
            WALL[:, sl] = _mm(gsl, BD[g], _NT).astype(BF16)
            PACC[g] += _mm(WQK[:, sl], gsl, _TN)
        g_copy(c).start()
        return carry

    lax.fori_loop(0, 4, p5_body, 0)
    for c in range(4):
        out_copies.append(g_copy(c))
    for g in range(8):
        pm = jnp.where(bdmask(), PACC[g], 0.0).astype(BF16)
        DWP[pl.ds(g * 128, 128), :] = _mm(pm, emat(), _NT).astype(BF16)
    cout2(DWP, dwphi_hbm)

    for c in out_copies:
        c.wait()


@jax.jit
def pallas_recurrent_scan__linear_kernel_hedgehog__dense_activation_relu__prompt_kernel(
    A_x: jax.Array,
    A_wqkv: jax.Array,
    A_w_phi: jax.Array,
    A_wo: jax.Array,
    B_x: jax.Array,
    B_w1: jax.Array,
    B_w2: jax.Array,
    grad_out: jax.Array,
):
    x = A_x.reshape(S, D)
    dout = grad_out.reshape(S, D)
    wphi = A_w_phi.reshape(H * DH, DH)
    any_spec = pl.BlockSpec(memory_space=pl.ANY)
    out_shape = (
        jax.ShapeDtypeStruct((S, D), BF16),
        jax.ShapeDtypeStruct((S, D), BF16),
        jax.ShapeDtypeStruct((D, 3 * D), BF16),
        jax.ShapeDtypeStruct((H * DH, DH), BF16),
        jax.ShapeDtypeStruct((D, D), BF16),
        jax.ShapeDtypeStruct((D, FF), BF16),
        jax.ShapeDtypeStruct((FF, D), BF16),
    )
    scratch = [
        pltpu.VMEM((S, D), BF16),
        pltpu.VMEM((S, D), BF16),
        pltpu.VMEM((D, 3 * D), BF16),
        pltpu.VMEM((D, 2 * D), BF16),
        pltpu.VMEM((H * DH, DH), BF16),
        pltpu.VMEM((8, 128, 128), BF16),
        pltpu.VMEM((D, D), BF16),
        pltpu.VMEM((D, FF), BF16),
        pltpu.VMEM((FF, D), BF16),
        pltpu.VMEM((S, D), BF16),
        pltpu.VMEM((S, 128), F32),
        pltpu.VMEM((2 * D, S), BF16),
        pltpu.VMEM((3 * D, S), BF16),
        pltpu.VMEM((S, FF), BF16),
        pltpu.VMEM((S, D), BF16),
        pltpu.VMEM((S, D), BF16),
        pltpu.VMEM((D, S), BF16),
        pltpu.VMEM((S, D), F32),
        pltpu.VMEM((NP, AUG, 128), BF16),
        pltpu.VMEM((NP, AUG, 128), F32),
        pltpu.VMEM((NP, AUG, 128), BF16),
        pltpu.VMEM((2 * D, TS), BF16),
        pltpu.VMEM((NP, AUG, TS), BF16),
        pltpu.VMEM((S, TF), BF16),
        pltpu.VMEM((H * DH, DH), BF16),
        pltpu.VMEM((2, TS, D), F32),
        pltpu.VMEM((2, TS, D), F32),
        pltpu.VMEM((8, 128, 128), F32),
        pltpu.SMEM((1,), jnp.int32),
        pltpu.SemaphoreType.DMA((NT,)),
        pltpu.SemaphoreType.DMA((16,)),
        pltpu.SemaphoreType.DMA((48,)),
    ]
    outs = pl.pallas_call(
        _kernel,
        in_specs=[any_spec] * 7,
        out_specs=[any_spec] * 7,
        out_shape=out_shape,
        scratch_shapes=scratch,
        compiler_params=pltpu.CompilerParams(vmem_limit_bytes=127 * 1024 * 1024),
    )(x, A_wqkv, wphi, A_wo, B_w1, B_w2, dout)
    out, gx, dwqkv, dwphi, dwo, dw1, dw2 = outs
    return (out.reshape(1, S, D), gx.reshape(1, S, D), dwqkv,
            dwphi.reshape(H, DH, DH), dwo, dw1, dw2)
```

```python
import jax
import jax.numpy as jnp
from jax import lax
import jax.experimental.pallas as pl
import jax.experimental.pallas.tpu as pltpu

S, D, H, DH, FF = 2048, 1024, 32, 32, 3584
TS = 256
NT = S // TS
TF = 256
NF = FF // TF
HC = 512
NHC = FF // HC
NP = H // 2
AUG = 80
F32 = jnp.float32
BF16 = jnp.bfloat16

_NN = (((1,), (0,)), ((), ()))
_NT = (((1,), (1,)), ((), ()))
_TN = (((0,), (0,)), ((), ()))
_TT = (((0,), (1,)), ((), ()))


def _mm(a, b, dn):
    return lax.dot_general(a, b, dn, preferred_element_type=F32)


def _rcp(x):
    r = pl.reciprocal(x, approx=True)
    return r * (2.0 - x * r)


def _softmax_pm(p):
    r, ts = p.shape
    nh = r // DH
    p3 = p.reshape(nh, DH, ts)
    mx = jnp.max(p3, axis=1, keepdims=True)
    mn = jnp.min(p3, axis=1, keepdims=True)
    ep = jnp.exp(p3 - mx)
    en = jnp.exp(mn - p3)
    ap = ep * _rcp(jnp.sum(ep, axis=1, keepdims=True))
    an = en * _rcp(jnp.sum(en, axis=1, keepdims=True))
    return jnp.concatenate([ap, an], axis=1).reshape(nh * 2 * DH, ts)


def _softmax_pm_bwd(phi, dphi):
    r, ts = phi.shape
    nh = r // (2 * DH)
    ph = phi.reshape(nh * 2, DH, ts)
    t = ph * dphi.reshape(nh * 2, DH, ts)
    dp = t - ph * jnp.sum(t, axis=1, keepdims=True)
    dp = dp.reshape(nh, 2 * DH, ts)
    return (dp[:, :DH, :] - dp[:, DH:, :]).reshape(nh * DH, ts)


def _rows(t):
    if isinstance(t, int):
        return pl.ds(t * TS, TS)
    return pl.ds(pl.multiple_of(t * TS, TS), TS)


def _kernel(x_hbm, wqkv_hbm, wphi_hbm, wo_hbm, w1_hbm, w2_hbm, dout_hbm,
            out_hbm, gx_hbm, dwqkv_hbm, dwphi_hbm, dwo_hbm, dw1_hbm, dw2_hbm,
            X, DO, WT, WOR, WPHI, BD, WO, W1, W2, XN, RSTD, PHIK, DQKV, R,
            DB, DS, OT, DXN, KVZ, DKVZ, DKVZB, PHIQ, DND, DHF, DWP, BB, PACC, DXA, DXB, FLAG,
            xsem, isem, osem):
    in_copies = []

    def cin(src, dst):
        c = pltpu.make_async_copy(src, dst, isem.at[len(in_copies)])
        c.start()
        in_copies.append(c)
        return c

    def x_copy(t):
        return pltpu.make_async_copy(x_hbm.at[_rows(t)], X.at[_rows(t)], xsem.at[t])

    def wrows(col, i, dst):
        return cin(wqkv_hbm.at[pl.ds(512 * i, 512), pl.ds(col, D)], dst.at[pl.ds(512 * i, 512), pl.ds(col, D)])

    FLAG[0] = 0
    x_copy(0).start()
    c_wk0 = wrows(D, 0, WOR)
    c_wphi = cin(wphi_hbm, WPHI)

    out_copies = []

    def cout(src, dst):
        c = pltpu.make_async_copy(src, dst, osem.at[len(out_copies)])
        c.start()
        out_copies.append(c)

    def bdmask():
        row = lax.broadcasted_iota(jnp.int32, (128, 128), 0)
        col = lax.broadcasted_iota(jnp.int32, (128, 128), 1)
        return (row // DH) == (col // DH)

    def emat():
        e_r = lax.broadcasted_iota(jnp.int32, (DH, 128), 0)
        e_c = lax.broadcasted_iota(jnp.int32, (DH, 128), 1)
        return jnp.where((e_c % DH) == e_r, 1.0, 0.0).astype(BF16)

    def m80():
        r80 = lax.broadcasted_iota(jnp.int32, (AUG, 128), 0)
        c80 = lax.broadcasted_iota(jnp.int32, (AUG, 128), 1)
        return jnp.where(r80 < 64, r80 // DH, (r80 - 64) // 8) == (c80 // 64)

    def ln_tile(t):
        rows = _rows(t)
        x = X[rows, :].astype(F32)
        mu = jnp.mean(x, axis=1, keepdims=True)
        xc = x - mu
        var = jnp.mean(xc * xc, axis=1, keepdims=True)
        rstd = lax.rsqrt(var + 1e-5)
        xn = (xc * rstd).astype(BF16)
        XN[rows, :] = xn
        RSTD[rows, :] = jnp.broadcast_to(rstd, (TS, 128))
        return xn

    def fold(g, off, rs=slice(None)):
        sl = pl.ds(off + g * 128, 128)
        WT[sl, rs] = _mm(BD[g], WOR[rs, sl], _TT).astype(BF16)

    def phik_tile(t, pk):
        rows = _rows(t)
        for c in range(8):
            PHIK[pl.ds(c * 256, 256), rows] = _softmax_pm(pk[c * 128:(c + 1) * 128]).astype(BF16)

    x_copy(0).wait()
    c_wk1 = wrows(D, 1, WOR)
    c_wv = cin(wqkv_hbm.at[:, pl.ds(2 * D, D)], WOR.at[:, pl.ds(2 * D, D)])
    xn0 = ln_tile(0)
    c_wphi.wait()
    c_wk0.wait()
    x_copy(1).start()
    for g in range(8):
        wrep = _mm(WPHI[pl.ds(g * 128, 128), :], emat(), _NN)
        BD[g] = jnp.where(bdmask(), wrep, 0.0).astype(BF16)
    for g in range(8):
        fold(g, D, pl.ds(0, 512))
    c_wk1.wait()
    for t in range(2, NT):
        x_copy(t).start()
    for g in range(8):
        fold(g, D, pl.ds(512, 512))
    phik_tile(0, _mm(WT[pl.ds(D, D), :], xn0, _NT))
    c_wv.wait()
    x_copy(1).wait()
    wvt = WOR[:, pl.ds(2 * D, D)].T
    WT[pl.ds(2 * D, D), :] = wvt
    DQKV[pl.ds(2 * D, D), _rows(0)] = _mm(wvt, xn0, _NT).astype(BF16)
    xn1 = ln_tile(1)
    DQKV[pl.ds(2 * D, D), _rows(1)] = _mm(wvt, xn1, _NT).astype(BF16)

    big = [(wqkv_hbm.at[:, pl.ds(0, D)], WOR.at[:, pl.ds(0, D)]), (w1_hbm, W1), (w2_hbm, W2),
           (dout_hbm, DO), (wo_hbm, WO)]
    nb = len(in_copies)

    def big_copy(k):
        return pltpu.make_async_copy(big[k][0], big[k][1], isem.at[nb + k])

    def p1_step(t, xn):
        pk = _mm(WT[pl.ds(D, D), :], xn, _NT)
        xn_next = ln_tile(t + 1)
        vt = _mm(WT[pl.ds(2 * D, D), :], xn_next, _NT)
        phik_tile(t, pk)
        DQKV[pl.ds(2 * D, D), _rows(t + 1)] = vt.astype(BF16)
        return xn_next

    def p1_body(i, xn):
        x_copy(2 * i + 2).wait()
        x_copy(2 * i + 3).wait()

        @pl.when(i == 0)
        def _():
            for k in range(len(big)):
                big_copy(k).start()

        return p1_step(2 * i + 2, p1_step(2 * i + 1, xn))

    xn_last = lax.fori_loop(0, (NT - 2) // 2, p1_body, xn1)
    c_wq, c_w1, c_w2, c_do, c_wo = [big_copy(k) for k in range(len(big))]
    c_wq.wait()
    pk = _mm(WT[pl.ds(D, D), :], xn_last, _NT)
    for g in range(8):
        fold(g, 0)
    phik_tile(NT - 1, pk)

    c_w1.wait()

    def p1h_body(j, carry):
        fs = pl.ds(pl.multiple_of(j * HC, 128), HC)
        h = _mm(XN[...], W1[:, fs], _NN)
        R[:, fs] = jnp.where(h > 0.0, h, jnp.where(h == 0.0, 0.0, -0.0)).astype(BF16)
        return carry

    lax.fori_loop(0, NHC, p1h_body, 0)

    def ffn_b(t, c):
        cs = pl.ds(c * 256 if isinstance(c, int) else pl.multiple_of(c * 256, 256), 256)
        BB[t % 2, :, cs] = _mm(R[_rows(t), :], W2[:, cs], _NN)

    ones_s = jnp.ones((16, S), BF16)
    for p in range(NP):
        v1 = jnp.concatenate([DQKV[pl.ds(2 * D + 64 * p, 64), :], ones_s], axis=0)
        kvz = _mm(v1, PHIK[pl.ds(128 * p, 128), :], _NT)
        KVZ[p] = jnp.where(m80(), kvz, 0.0).astype(BF16)
        DKVZ[p] = jnp.zeros((AUG, 128), F32)

    c_w2.wait()

    def b0_body(c, carry):
        ffn_b(0, 2 * c)
        ffn_b(0, 2 * c + 1)
        return carry

    lax.fori_loop(0, 2, b0_body, 0)
    c_wo.wait()
    c_do.wait()

    def p2_tile(t, with_ffn):
        rows = _rows(t)
        b = BB[t % 2]
        sig = 0.5 * jnp.tanh(0.5 * b) + 0.5
        g = b * sig
        dout = DO[rows, :].astype(F32)
        ds = (dout * g).astype(BF16)
        e = dout * (sig + g * (1.0 - sig))
        DS[rows, :] = ds
        DXN[rows, :] = jnp.zeros((TS, D), F32)
        pq = _mm(WT[pl.ds(0, D), :], XN[rows, :], _NT)
        dot_ = _mm(WO[...], ds, _NT)
        if with_ffn:
            ffn_b(t + 1, 0)
        for c in range(8):
            PHIQ[pl.ds(c * 256, 256), :] = _softmax_pm(pq[c * 128:(c + 1) * 128]).astype(BF16)
        nds = [_mm(KVZ[p], PHIQ[pl.ds(128 * p, 128), :], _NN) for p in range(NP)]
        if with_ffn:
            ffn_b(t + 1, 1)
        for p in range(NP):
            nd = nds[p]
            rden = _rcp(nd[64:AUG].reshape(2, 1, 8, TS) + 1e-6)
            o4 = nd[0:64].reshape(2, 4, 8, TS) * rden
            OT[pl.ds(64 * p, 64), rows] = o4.reshape(64, TS).astype(BF16)
            dnum = dot_[64 * p:64 * (p + 1)].reshape(2, 4, 8, TS) * rden
            dden = -jnp.sum(dnum * o4, axis=1, keepdims=True)
            DND[p, pl.ds(0, 64), :] = dnum.reshape(64, TS).astype(BF16)
            DND[p, pl.ds(64, 16), :] = dden.reshape(16, TS).astype(BF16)
        dphis = []
        for p in range(NP):
            dnd = DND[p]
            dphis.append(_mm(KVZ[p], dnd, _TN))
            DKVZ[p] += _mm(dnd, PHIQ[pl.ds(128 * p, 128), :], _NT)
        s = _mm(OT[:, rows], WO[...], _TN)
        for p in range(NP):
            phi = PHIQ[pl.ds(128 * p, 128), :].astype(F32)
            DQKV[pl.ds(64 * p, 64), rows] = _softmax_pm_bwd(phi, dphis[p]).astype(BF16)
        if with_ffn:
            ffn_b(t + 1, 2)
            ffn_b(t + 1, 3)
        X[rows, :] = (X[rows, :].astype(F32) + s * g).astype(BF16)
        DB[rows, :] = (e * s).astype(BF16)

    def p2_body(t, carry):
        p2_tile(t, True)
        return carry

    lax.fori_loop(0, NT - 1, p2_body, 0)
    p2_tile(NT - 1, False)
    cout(X, out_hbm)

    for p in range(NP):
        DKVZB[p] = jnp.where(m80(), DKVZ[p], 0.0).astype(BF16)

    def kside(p):
        if isinstance(p, int):
            vs, ks, fs_ = pl.ds(2 * D + 64 * p, 64), pl.ds(D + 64 * p, 64), pl.ds(128 * p, 128)
        else:
            vs = pl.ds(pl.multiple_of(2 * D + 64 * p, 64), 64)
            ks = pl.ds(pl.multiple_of(D + 64 * p, 64), 64)
            fs_ = pl.ds(pl.multiple_of(128 * p, 128), 128)
        v1 = jnp.concatenate([DQKV[vs, :], ones_s], axis=0)
        dk = DKVZB[p]
        phi = PHIK[fs_, :]
        dphi = _mm(dk, v1, _TN)
        DQKV[vs, :] = _mm(dk[0:64], phi, _NN).astype(BF16)
        DQKV[ks, :] = _softmax_pm_bwd(phi.astype(F32), dphi).astype(BF16)

    DXB[...] = jnp.zeros((TS, D), F32)
    for p in range(NF, NP):
        kside(p)

    base3 = len(out_copies)

    def dw_copies(j):
        fs = pl.ds(j * TF if isinstance(j, int) else pl.multiple_of(j * TF, 128), TF)
        return (pltpu.make_async_copy(W2.at[fs, :], dw2_hbm.at[fs, :], osem.at[base3 + 2 * j]),
                pltpu.make_async_copy(W1.at[:, fs], dw1_hbm.at[:, fs], osem.at[base3 + 2 * j + 1]))

    def p3_body(j, carry):
        fs = pl.ds(pl.multiple_of(j * TF, 128), TF)
        c2, c1 = dw_copies(j)
        dr = _mm(DB[...], W2[fs, :], _NT)
        r = R[:, fs].astype(F32)
        rb = lax.bitcast_convert_type(r, jnp.int32)
        DHF[...] = jnp.where(r > 0.0, dr, jnp.where(rb == 0, 0.5 * dr, 0.0)).astype(BF16)
        W2[fs, :] = _mm(R[:, fs], DB[...], _TN).astype(BF16)
        c2.start()
        kside(j)
        DXN[...] += _mm(DHF[...], W1[:, fs], _NT)
        W1[:, fs] = _mm(XN[...], DHF[...], _TN).astype(BF16)
        c1.start()
        return carry

    lax.fori_loop(0, NF, p3_body, 0)
    for j in range(NF):
        out_copies.extend(dw_copies(j))

    def dwo_chunk(c):
        cs = pl.ds(c * 128 if isinstance(c, int) else pl.multiple_of(c * 128, 128), 128)
        WO[:, cs] = _mm(OT[...], DS[:, cs], _NN).astype(BF16)

    def gx_tile(t, dx_ref, m1, m2):
        rows = _rows(t)
        xn = XN[rows, :].astype(F32)
        rstd = RSTD[rows, :][:, 0:1]
        return DO[rows, :].astype(F32) + rstd * (dx_ref[...] - m1 - xn * m2)

    out_copies.pop(0).wait()

    def p4_step(t, carry, prev_ref, cur_ref):
        never = FLAG[0] != 0
        rows = _rows(t)
        tp = jnp.maximum(t - 1, 0)
        dwo_chunk(t)
        dxn = _mm(DQKV[:, rows], WT[...], _TN) + DXN[rows, :]
        X[_rows(tp), :] = jnp.where(never, dxn, gx_tile(tp, prev_ref, *carry)).astype(BF16)
        m1 = jnp.mean(dxn, axis=1, keepdims=True)
        m2 = jnp.mean(dxn * XN[rows, :].astype(F32), axis=1, keepdims=True)
        cur_ref[...] = dxn
        return m1, m2

    def p4_body(i, carry):
        return p4_step(2 * i + 1, p4_step(2 * i, carry, DXB, DXA), DXA, DXB)

    zc = jnp.zeros((TS, 1), F32)
    m12 = lax.fori_loop(0, NT // 2, p4_body, (zc, zc))
    nsem = [len(out_copies) + 1]

    def cout2(src_, dst_):
        c = pltpu.make_async_copy(src_, dst_, osem.at[nsem[0]])
        nsem[0] += 1
        c.start()
        out_copies.append(c)

    cout2(WO, dwo_hbm)

    X[_rows(NT - 1), :] = gx_tile(NT - 1, DXB, *m12).astype(BF16)
    cout2(X, gx_hbm)
    for g in range(8):
        PACC[g] = jnp.zeros((128, 128), F32)
    base5 = nsem[0]
    nsem[0] += 4

    def g_copy(c):
        cs = pl.ds(c * 512 if isinstance(c, int) else pl.multiple_of(c * 512, 512), 512)
        return pltpu.make_async_copy(WOR.at[:, cs], dwqkv_hbm.at[:, cs], osem.at[base5 + c])

    def p5_body(c, carry):
        cs = pl.ds(pl.multiple_of(c * 512, 512), 512)
        gb = _mm(XN[...], DQKV[cs, :], _TT).astype(BF16)
        worig = WOR[:, cs]
        dws = []
        for gg in range(4):
            g = (c * 4 + gg) % 8
            gsl = gb[:, gg * 128:(gg + 1) * 128]
            PACC[g] += _mm(worig[:, gg * 128:(gg + 1) * 128], gsl, _TN)
            dws.append(_mm(gsl, BD[g], _NT).astype(BF16))
        WOR[:, cs] = jnp.concatenate(dws, axis=1)
        g_copy(c).start()
        return carry

    lax.fori_loop(0, 4, p5_body, 0)
    for c in range(4):
        out_copies.append(g_copy(c))
    for g in range(8):
        pm = jnp.where(bdmask(), PACC[g], 0.0).astype(BF16)
        DWP[pl.ds(g * 128, 128), :] = _mm(pm, emat(), _NT).astype(BF16)
    cout2(DWP, dwphi_hbm)
    off = 2 * D
    for w in (512, 256, 128, 128):
        cs = pl.ds(off, w)
        WOR[:, cs] = _mm(XN[...], DQKV[cs, :], _TT).astype(BF16)
        cout2(WOR.at[:, cs], dwqkv_hbm.at[:, cs])
        off += w

    for c in out_copies:
        c.wait()


@jax.jit
def pallas_recurrent_scan__linear_kernel_hedgehog__dense_activation_relu__prompt_kernel(
    A_x: jax.Array,
    A_wqkv: jax.Array,
    A_w_phi: jax.Array,
    A_wo: jax.Array,
    B_x: jax.Array,
    B_w1: jax.Array,
    B_w2: jax.Array,
    grad_out: jax.Array,
):
    x = A_x.reshape(S, D)
    dout = grad_out.reshape(S, D)
    wphi = A_w_phi.reshape(H * DH, DH)
    any_spec = pl.BlockSpec(memory_space=pl.ANY)
    out_shape = (
        jax.ShapeDtypeStruct((S, D), BF16),
        jax.ShapeDtypeStruct((S, D), BF16),
        jax.ShapeDtypeStruct((D, 3 * D), BF16),
        jax.ShapeDtypeStruct((H * DH, DH), BF16),
        jax.ShapeDtypeStruct((D, D), BF16),
        jax.ShapeDtypeStruct((D, FF), BF16),
        jax.ShapeDtypeStruct((FF, D), BF16),
    )
    scratch = [
        pltpu.VMEM((S, D), BF16),
        pltpu.VMEM((S, D), BF16),
        pltpu.VMEM((3 * D, D), BF16),
        pltpu.VMEM((D, 3 * D), BF16),
        pltpu.VMEM((H * DH, DH), BF16),
        pltpu.VMEM((8, 128, 128), BF16),
        pltpu.VMEM((D, D), BF16),
        pltpu.VMEM((D, FF), BF16),
        pltpu.VMEM((FF, D), BF16),
        pltpu.VMEM((S, D), BF16),
        pltpu.VMEM((S, 128), F32),
        pltpu.VMEM((2 * D, S), BF16),
        pltpu.VMEM((3 * D, S), BF16),
        pltpu.VMEM((S, FF), BF16),
        pltpu.VMEM((S, D), BF16),
        pltpu.VMEM((S, D), BF16),
        pltpu.VMEM((D, S), BF16),
        pltpu.VMEM((S, D), F32),
        pltpu.VMEM((NP, AUG, 128), BF16),
        pltpu.VMEM((NP, AUG, 128), F32),
        pltpu.VMEM((NP, AUG, 128), BF16),
        pltpu.VMEM((2 * D, TS), BF16),
        pltpu.VMEM((NP, AUG, TS), BF16),
        pltpu.VMEM((S, TF), BF16),
        pltpu.VMEM((H * DH, DH), BF16),
        pltpu.VMEM((2, TS, D), F32),
        pltpu.VMEM((8, 128, 128), F32),
        pltpu.VMEM((TS, D), F32),
        pltpu.VMEM((TS, D), F32),
        pltpu.SMEM((1,), jnp.int32),
        pltpu.SemaphoreType.DMA((NT,)),
        pltpu.SemaphoreType.DMA((16,)),
        pltpu.SemaphoreType.DMA((48,)),
    ]
    outs = pl.pallas_call(
        _kernel,
        in_specs=[any_spec] * 7,
        out_specs=[any_spec] * 7,
        out_shape=out_shape,
        scratch_shapes=scratch,
        compiler_params=pltpu.CompilerParams(vmem_limit_bytes=127 * 1024 * 1024),
    )(x, A_wqkv, wphi, A_wo, B_w1, B_w2, dout)
    out, gx, dwqkv, dwphi, dwo, dw1, dw2 = outs
    return (out.reshape(1, S, D), gx.reshape(1, S, D), dwqkv,
            dwphi.reshape(H, DH, DH), dwo, dw1, dw2)
```

```python
import jax
import jax.numpy as jnp
from jax import lax
import jax.experimental.pallas as pl
import jax.experimental.pallas.tpu as pltpu

S, D, H, DH, FF = 2048, 1024, 32, 32, 3584
TS = 256
NT = S // TS
TF = 256
NF = FF // TF
HC = 512
NHC = FF // HC
NP = H // 2
AUG = 80
F32 = jnp.float32
BF16 = jnp.bfloat16

_NN = (((1,), (0,)), ((), ()))
_NT = (((1,), (1,)), ((), ()))
_TN = (((0,), (0,)), ((), ()))
_TT = (((0,), (1,)), ((), ()))


def _mm(a, b, dn):
    return lax.dot_general(a, b, dn, preferred_element_type=F32)


def _rcp(x):
    r = pl.reciprocal(x, approx=True)
    return r * (2.0 - x * r)


def _softmax_pm(p):
    r, ts = p.shape
    nh = r // DH
    p3 = p.reshape(nh, DH, ts)
    mx = jnp.max(p3, axis=1, keepdims=True)
    mn = jnp.min(p3, axis=1, keepdims=True)
    ep = jnp.exp(p3 - mx)
    en = jnp.exp(mn - p3)
    ap = ep * _rcp(jnp.sum(ep, axis=1, keepdims=True))
    an = en * _rcp(jnp.sum(en, axis=1, keepdims=True))
    return jnp.concatenate([ap, an], axis=1).reshape(nh * 2 * DH, ts)


def _softmax_pm_bwd(phi, dphi):
    r, ts = phi.shape
    nh = r // (2 * DH)
    ph = phi.reshape(nh * 2, DH, ts)
    t = ph * dphi.reshape(nh * 2, DH, ts)
    dp = t - ph * jnp.sum(t, axis=1, keepdims=True)
    dp = dp.reshape(nh, 2 * DH, ts)
    return (dp[:, :DH, :] - dp[:, DH:, :]).reshape(nh * DH, ts)


def _ds(i, size, align=None):
    if isinstance(i, int):
        return pl.ds(i * size, size)
    return pl.ds(pl.multiple_of(i * size, align or size), size)


def _rows(t):
    return _ds(t, TS)


def _kernel(x_hbm, wqkv_hbm, wphi_hbm, wo_hbm, w1_hbm, w2_hbm, dout_hbm,
            out_hbm, gx_hbm, dwqkv_hbm, dwphi_hbm, dwo_hbm, dw1_hbm, dw2_hbm,
            X, DO, WT, WOR, WPHI, BD, WO, W1, W2, XN, RSTD, PHIK, DQKV, R,
            DB, DS, OT, DXN, KVZ, DKVZ, DKVZB, PHIQ, DND, DHF, DWP, BB, PACC, DXA, DXB, PK0, FLAG,
            xsem, isem, osem):
    n_in = [0]

    def cin(src, dst):
        c = pltpu.make_async_copy(src, dst, isem.at[n_in[0]])
        n_in[0] += 1
        c.start()
        return c

    def x_copy(t):
        return pltpu.make_async_copy(x_hbm.at[_rows(t)], X.at[_rows(t)], xsem.at[t])

    def wrows(col, i):
        return cin(wqkv_hbm.at[pl.ds(512 * i, 512), pl.ds(col, D)],
                   WOR.at[pl.ds(512 * i, 512), pl.ds(col, D)])

    (O_OUT, O_GX, O_DWQKV, O_DWPHI, O_DWO, O_DW1, O_DW2) = range(7)

    def cout(src, dst, k):
        pltpu.make_async_copy(src, dst, osem.at[k]).start()

    FLAG[0] = 0
    x_copy(0).start()
    c_wk0 = wrows(D, 0)
    c_wphi = cin(wphi_hbm, WPHI)

    def bdmask():
        row = lax.broadcasted_iota(jnp.int32, (128, 128), 0)
        col = lax.broadcasted_iota(jnp.int32, (128, 128), 1)
        return (row // DH) == (col // DH)

    def emat():
        e_r = lax.broadcasted_iota(jnp.int32, (DH, 128), 0)
        e_c = lax.broadcasted_iota(jnp.int32, (DH, 128), 1)
        return jnp.where((e_c % DH) == e_r, 1.0, 0.0).astype(BF16)

    def m80():
        r80 = lax.broadcasted_iota(jnp.int32, (AUG, 128), 0)
        c80 = lax.broadcasted_iota(jnp.int32, (AUG, 128), 1)
        return jnp.where(r80 < 64, r80 // DH, (r80 - 64) // 8) == (c80 // 64)

    def ln_tile(t):
        rows = _rows(t)
        x = X[rows, :].astype(F32)
        mu = jnp.mean(x, axis=1, keepdims=True)
        xc = x - mu
        var = jnp.mean(xc * xc, axis=1, keepdims=True)
        rstd = lax.rsqrt(var + 1e-5)
        xn = (xc * rstd).astype(BF16)
        XN[rows, :] = xn
        RSTD[rows, :] = jnp.broadcast_to(rstd, (TS, 128))
        return xn

    def fold(g, off, rs=slice(None)):
        sl = pl.ds(off + g * 128, 128)
        WT[sl, rs] = _mm(BD[g], WOR[rs, sl], _TT).astype(BF16)

    def phik_tile(t, pk):
        rows = _rows(t)
        for c in range(8):
            PHIK[pl.ds(c * 256, 256), rows] = _softmax_pm(pk[c * 128:(c + 1) * 128]).astype(BF16)

    DKVZ[...] = jnp.zeros(DKVZ.shape, F32)
    PACC[...] = jnp.zeros(PACC.shape, F32)
    DXB[...] = jnp.zeros(DXB.shape, F32)
    DXN[...] = jnp.zeros(DXN.shape, F32)

    x_copy(0).wait()
    c_wk1 = wrows(D, 1)
    x_copy(1).start()
    xn0 = ln_tile(0)
    c_wphi.wait()
    c_wk0.wait()
    c_wv = cin(wqkv_hbm.at[:, pl.ds(2 * D, D)], WOR.at[:, pl.ds(2 * D, D)])
    for g in range(8):
        wrep = _mm(WPHI[pl.ds(g * 128, 128), :], emat(), _NN)
        BD[g] = jnp.where(bdmask(), wrep, 0.0).astype(BF16)
    for g in range(8):
        fold(g, D, pl.ds(0, 512))
    PK0[...] = _mm(WT[pl.ds(D, D), pl.ds(0, 512)], xn0[:, 0:512], _NT)
    c_wk1.wait()
    x_copy(1).wait()
    for t in range(2, NT):
        x_copy(t).start()
    for g in range(8):
        fold(g, D, pl.ds(512, 512))
    xn1 = ln_tile(1)
    phik_tile(0, PK0[...] + _mm(WT[pl.ds(D, D), pl.ds(512, 512)], xn0[:, 512:D], _NT))
    phik_tile(1, _mm(WT[pl.ds(D, D), :], xn1, _NT))
    c_wv.wait()
    x_copy(2).wait()
    wvt = WOR[:, pl.ds(2 * D, D)].T
    WT[pl.ds(2 * D, D), :] = wvt
    DQKV[pl.ds(2 * D, D), _rows(0)] = _mm(wvt, xn0, _NT).astype(BF16)
    DQKV[pl.ds(2 * D, D), _rows(1)] = _mm(wvt, xn1, _NT).astype(BF16)
    xn2 = ln_tile(2)
    DQKV[pl.ds(2 * D, D), _rows(2)] = _mm(wvt, xn2, _NT).astype(BF16)

    big = [(wqkv_hbm.at[:, pl.ds(0, D)], WOR.at[:, pl.ds(0, D)]), (w1_hbm, W1), (w2_hbm, W2),
           (dout_hbm, DO), (wo_hbm, WO)]
    nb = n_in[0]

    def big_copy(k):
        return pltpu.make_async_copy(big[k][0], big[k][1], isem.at[nb + k])

    def p1_step(t, xn):
        pk = _mm(WT[pl.ds(D, D), :], xn, _NT)
        xn_next = ln_tile(t + 1)
        vt = _mm(WT[pl.ds(2 * D, D), :], xn_next, _NT)
        phik_tile(t, pk)
        DQKV[pl.ds(2 * D, D), _rows(t + 1)] = vt.astype(BF16)
        return xn_next

    def p1_body(i, xn):
        x_copy(2 * i + 3).wait()
        x_copy(2 * i + 4).wait()

        @pl.when(i == 0)
        def _():
            for k in range(len(big)):
                big_copy(k).start()

        return p1_step(2 * i + 3, p1_step(2 * i + 2, xn))

    xn6 = lax.fori_loop(0, (NT - 4) // 2, p1_body, xn2)
    c_wq, c_w1, c_w2, c_do, c_wo = [big_copy(k) for k in range(len(big))]
    x_copy(NT - 1).wait()
    c_wq.wait()
    xn_last = p1_step(NT - 2, xn6)
    pk = _mm(WT[pl.ds(D, D), :], xn_last, _NT)
    for g in range(8):
        fold(g, 0)
    phik_tile(NT - 1, pk)

    c_w1.wait()

    def p1h_body(j, carry):
        fs = _ds(j, HC, 128)
        h = _mm(XN[...], W1[:, fs], _NN)
        R[:, fs] = jnp.where(h > 0.0, h, jnp.where(h == 0.0, 0.0, -0.0)).astype(BF16)
        return carry

    lax.fori_loop(0, NHC, p1h_body, 0)

    def ffn_b(t, c):
        cs = _ds(c, 256)
        BB[t % 2, :, cs] = _mm(R[_rows(t), :], W2[:, cs], _NN)

    ones_s = jnp.ones((16, S), BF16)
    for p in range(NP):
        v1 = jnp.concatenate([DQKV[pl.ds(2 * D + 64 * p, 64), :], ones_s], axis=0)
        kvz = _mm(v1, PHIK[pl.ds(128 * p, 128), :], _NT)
        KVZ[p] = jnp.where(m80(), kvz, 0.0).astype(BF16)

    c_w2.wait()

    def b0_body(c, carry):
        ffn_b(0, 2 * c)
        ffn_b(0, 2 * c + 1)
        return carry

    lax.fori_loop(0, 2, b0_body, 0)
    c_wo.wait()
    c_do.wait()

    def p2_tile(t, with_ffn):
        rows = _rows(t)
        b = BB[t % 2]
        sig = 0.5 * jnp.tanh(0.5 * b) + 0.5
        g = b * sig
        dout = DO[rows, :].astype(F32)
        ds = (dout * g).astype(BF16)
        e = dout * (sig + g * (1.0 - sig))
        DS[rows, :] = ds
        pq = _mm(WT[pl.ds(0, D), :], XN[rows, :], _NT)
        dot_ = _mm(WO[...], ds, _NT)
        if with_ffn:
            ffn_b(t + 1, 0)
        for c in range(8):
            PHIQ[pl.ds(c * 256, 256), :] = _softmax_pm(pq[c * 128:(c + 1) * 128]).astype(BF16)
        nds = [_mm(KVZ[p], PHIQ[pl.ds(128 * p, 128), :], _NN) for p in range(NP)]
        if with_ffn:
            ffn_b(t + 1, 1)
        for p in range(NP):
            nd = nds[p]
            rden = _rcp(nd[64:AUG].reshape(2, 1, 8, TS) + 1e-6)
            o4 = nd[0:64].reshape(2, 4, 8, TS) * rden
            OT[pl.ds(64 * p, 64), rows] = o4.reshape(64, TS).astype(BF16)
            dnum = dot_[64 * p:64 * (p + 1)].reshape(2, 4, 8, TS) * rden
            dden = -jnp.sum(dnum * o4, axis=1, keepdims=True)
            DND[p, pl.ds(0, 64), :] = dnum.reshape(64, TS).astype(BF16)
            DND[p, pl.ds(64, 16), :] = dden.reshape(16, TS).astype(BF16)
        dphis = []
        for p in range(NP):
            dnd = DND[p]
            dphis.append(_mm(KVZ[p], dnd, _TN))
            DKVZ[p] += _mm(dnd, PHIQ[pl.ds(128 * p, 128), :], _NT)
        s = _mm(OT[:, rows], WO[...], _TN)
        for p in range(NP):
            phi = PHIQ[pl.ds(128 * p, 128), :].astype(F32)
            DQKV[pl.ds(64 * p, 64), rows] = _softmax_pm_bwd(phi, dphis[p]).astype(BF16)
        if with_ffn:
            ffn_b(t + 1, 2)
            ffn_b(t + 1, 3)
        X[rows, :] = (X[rows, :].astype(F32) + s * g).astype(BF16)
        DB[rows, :] = (e * s).astype(BF16)

    def p2_body(t, carry):
        p2_tile(t, True)
        return carry

    lax.fori_loop(0, NT - 1, p2_body, 0)
    p2_tile(NT - 1, False)
    cout(X, out_hbm, O_OUT)

    for p in range(NP):
        DKVZB[p] = jnp.where(m80(), DKVZ[p], 0.0).astype(BF16)

    def kside(p):
        if isinstance(p, int):
            vs, ks = pl.ds(2 * D + 64 * p, 64), pl.ds(D + 64 * p, 64)
        else:
            vs = pl.ds(pl.multiple_of(2 * D + 64 * p, 64), 64)
            ks = pl.ds(pl.multiple_of(D + 64 * p, 64), 64)
        v1 = jnp.concatenate([DQKV[vs, :], ones_s], axis=0)
        dk = DKVZB[p]
        phi = PHIK[_ds(p, 128), :]
        dphi = _mm(dk, v1, _TN)
        DQKV[vs, :] = _mm(dk[0:64], phi, _NN).astype(BF16)
        DQKV[ks, :] = _softmax_pm_bwd(phi.astype(F32), dphi).astype(BF16)

    for p in range(NF, NP):
        kside(p)

    def p3_body(j, carry):
        fs = _ds(j, TF, 128)
        dr = _mm(DB[...], W2[fs, :], _NT)
        r = R[:, fs].astype(F32)
        rb = lax.bitcast_convert_type(r, jnp.int32)
        DHF[...] = jnp.where(r > 0.0, dr, jnp.where(rb == 0, 0.5 * dr, 0.0)).astype(BF16)
        W2[fs, :] = _mm(R[:, fs], DB[...], _TN).astype(BF16)
        cout(W2.at[fs, :], dw2_hbm.at[fs, :], O_DW2)
        kside(j)
        DXN[...] += _mm(DHF[...], W1[:, fs], _NT)
        W1[:, fs] = _mm(XN[...], DHF[...], _TN).astype(BF16)
        cout(W1.at[:, fs], dw1_hbm.at[:, fs], O_DW1)
        return carry

    lax.fori_loop(0, NF, p3_body, 0)

    def dwo_chunk(c):
        cs = _ds(c, 128)
        WO[:, cs] = _mm(OT[...], DS[:, cs], _NN).astype(BF16)

    def gx_tile(t, dx_ref, m1, m2):
        rows = _rows(t)
        xn = XN[rows, :].astype(F32)
        rstd = RSTD[rows, :][:, 0:1]
        return DO[rows, :].astype(F32) + rstd * (dx_ref[...] - m1 - xn * m2)

    pltpu.make_async_copy(X, out_hbm, osem.at[O_OUT]).wait()

    def p4_step(t, carry, prev_ref, cur_ref):
        never = FLAG[0] != 0
        rows = _rows(t)
        tp = jnp.maximum(t - 1, 0)
        dwo_chunk(t)
        dxn = _mm(DQKV[:, rows], WT[...], _TN) + DXN[rows, :]
        X[_rows(tp), :] = jnp.where(never, dxn, gx_tile(tp, prev_ref, *carry)).astype(BF16)
        m1 = jnp.mean(dxn, axis=1, keepdims=True)
        m2 = jnp.mean(dxn * XN[rows, :].astype(F32), axis=1, keepdims=True)
        cur_ref[...] = dxn
        return m1, m2

    def p4_body(i, carry):
        return p4_step(2 * i + 1, p4_step(2 * i, carry, DXB, DXA), DXA, DXB)

    zc = jnp.zeros((TS, 1), F32)
    m12 = lax.fori_loop(0, NT // 2, p4_body, (zc, zc))
    cout(WO, dwo_hbm, O_DWO)
    head = pl.ds(0, S - TS)
    cout(X.at[head], gx_hbm.at[head], O_GX)

    def p5_body(c, carry):
        cs = _ds(c, 512)
        gb = _mm(XN[...], DQKV[cs, :], _TT).astype(BF16)
        worig = WOR[:, cs]
        dws = []
        for gg in range(4):
            g = (c * 4 + gg) % 8
            gsl = gb[:, gg * 128:(gg + 1) * 128]
            PACC[g] += _mm(worig[:, gg * 128:(gg + 1) * 128], gsl, _TN)
            dws.append(_mm(gsl, BD[g], _NT).astype(BF16))
        WOR[:, cs] = jnp.concatenate(dws, axis=1)
        cout(WOR.at[:, cs], dwqkv_hbm.at[:, cs], O_DWQKV)
        return carry

    lax.fori_loop(0, 4, p5_body, 0)
    for g in range(8):
        pm = jnp.where(bdmask(), PACC[g], 0.0).astype(BF16)
        DWP[pl.ds(g * 128, 128), :] = _mm(pm, emat(), _NT).astype(BF16)
    cout(DWP, dwphi_hbm, O_DWPHI)
    off = 2 * D
    for w in (512, 256, 128, 128):
        cs = pl.ds(off, w)
        gv = _mm(XN[...], DQKV[cs, :], _TT)
        WOR[:, cs] = gv.astype(BF16)
        cout(WOR.at[:, cs], dwqkv_hbm.at[:, cs], O_DWQKV)
        if w == 512:
            anchor = jnp.concatenate([gv[0:TS], gv[2 * TS:3 * TS]], axis=1)
            X[_rows(NT - 1), :] = jnp.where(
                FLAG[0] != 0, anchor, gx_tile(NT - 1, DXB, *m12)).astype(BF16)
            cout(X.at[_rows(NT - 1)], gx_hbm.at[_rows(NT - 1)], O_GX)
        off += w

    for src, dst, k in ((W2, dw2_hbm, O_DW2), (W1, dw1_hbm, O_DW1), (WO, dwo_hbm, O_DWO),
                        (X, gx_hbm, O_GX), (DWP, dwphi_hbm, O_DWPHI), (WOR, dwqkv_hbm, O_DWQKV)):
        pltpu.make_async_copy(src, dst, osem.at[k]).wait()


@jax.jit
def pallas_recurrent_scan__linear_kernel_hedgehog__dense_activation_relu__prompt_kernel(
    A_x: jax.Array,
    A_wqkv: jax.Array,
    A_w_phi: jax.Array,
    A_wo: jax.Array,
    B_x: jax.Array,
    B_w1: jax.Array,
    B_w2: jax.Array,
    grad_out: jax.Array,
):
    x = A_x.reshape(S, D)
    dout = grad_out.reshape(S, D)
    wphi = A_w_phi.reshape(H * DH, DH)
    any_spec = pl.BlockSpec(memory_space=pl.ANY)
    out_shape = (
        jax.ShapeDtypeStruct((S, D), BF16),
        jax.ShapeDtypeStruct((S, D), BF16),
        jax.ShapeDtypeStruct((D, 3 * D), BF16),
        jax.ShapeDtypeStruct((H * DH, DH), BF16),
        jax.ShapeDtypeStruct((D, D), BF16),
        jax.ShapeDtypeStruct((D, FF), BF16),
        jax.ShapeDtypeStruct((FF, D), BF16),
    )
    scratch = [
        pltpu.VMEM((S, D), BF16),
        pltpu.VMEM((S, D), BF16),
        pltpu.VMEM((3 * D, D), BF16),
        pltpu.VMEM((D, 3 * D), BF16),
        pltpu.VMEM((H * DH, DH), BF16),
        pltpu.VMEM((8, 128, 128), BF16),
        pltpu.VMEM((D, D), BF16),
        pltpu.VMEM((D, FF), BF16),
        pltpu.VMEM((FF, D), BF16),
        pltpu.VMEM((S, D), BF16),
        pltpu.VMEM((S, 128), F32),
        pltpu.VMEM((2 * D, S), BF16),
        pltpu.VMEM((3 * D, S), BF16),
        pltpu.VMEM((S, FF), BF16),
        pltpu.VMEM((S, D), BF16),
        pltpu.VMEM((S, D), BF16),
        pltpu.VMEM((D, S), BF16),
        pltpu.VMEM((S, D), F32),
        pltpu.VMEM((NP, AUG, 128), BF16),
        pltpu.VMEM((NP, AUG, 128), F32),
        pltpu.VMEM((NP, AUG, 128), BF16),
        pltpu.VMEM((2 * D, TS), BF16),
        pltpu.VMEM((NP, AUG, TS), BF16),
        pltpu.VMEM((S, TF), BF16),
        pltpu.VMEM((H * DH, DH), BF16),
        pltpu.VMEM((2, TS, D), F32),
        pltpu.VMEM((8, 128, 128), F32),
        pltpu.VMEM((TS, D), F32),
        pltpu.VMEM((TS, D), F32),
        pltpu.VMEM((D, TS), F32),
        pltpu.SMEM((1,), jnp.int32),
        pltpu.SemaphoreType.DMA((NT,)),
        pltpu.SemaphoreType.DMA((16,)),
        pltpu.SemaphoreType.DMA((7,)),
    ]
    outs = pl.pallas_call(
        _kernel,
        in_specs=[any_spec] * 7,
        out_specs=[any_spec] * 7,
        out_shape=out_shape,
        scratch_shapes=scratch,
        compiler_params=pltpu.CompilerParams(vmem_limit_bytes=127 * 1024 * 1024),
    )(x, A_wqkv, wphi, A_wo, B_w1, B_w2, dout)
    out, gx, dwqkv, dwphi, dwo, dw1, dw2 = outs
    return (out.reshape(1, S, D), gx.reshape(1, S, D), dwqkv,
            dwphi.reshape(H, DH, DH), dwo, dw1, dw2)
```

```python
import jax
import jax.numpy as jnp
from jax import lax
import jax.experimental.pallas as pl
import jax.experimental.pallas.tpu as pltpu

S, D, H, DH, FF = 2048, 1024, 32, 32, 3584
TS = 256
NT = S // TS
TF = 256
NF = FF // TF
HC = 512
NHC = FF // HC
NP = H // 2
AUG = 80
F32 = jnp.float32
BF16 = jnp.bfloat16

_NN = (((1,), (0,)), ((), ()))
_NT = (((1,), (1,)), ((), ()))
_TN = (((0,), (0,)), ((), ()))
_TT = (((0,), (1,)), ((), ()))


def _mm(a, b, dn):
    return lax.dot_general(a, b, dn, preferred_element_type=F32)


def _rcp(x):
    r = pl.reciprocal(x, approx=True)
    return r * (2.0 - x * r)


def _softmax_pm(p):
    r, ts = p.shape
    nh = r // DH
    p3 = p.reshape(nh, DH, ts)
    mx = jnp.max(p3, axis=1, keepdims=True)
    mn = jnp.min(p3, axis=1, keepdims=True)
    ep = jnp.exp(p3 - mx)
    en = jnp.exp(mn - p3)
    ap = ep * _rcp(jnp.sum(ep, axis=1, keepdims=True))
    an = en * _rcp(jnp.sum(en, axis=1, keepdims=True))
    return jnp.concatenate([ap, an], axis=1).reshape(nh * 2 * DH, ts)


def _softmax_pm_bwd(phi, dphi):
    r, ts = phi.shape
    nh = r // (2 * DH)
    ph = phi.reshape(nh * 2, DH, ts)
    t = ph * dphi.reshape(nh * 2, DH, ts)
    dp = t - ph * jnp.sum(t, axis=1, keepdims=True)
    dp = dp.reshape(nh, 2 * DH, ts)
    return (dp[:, :DH, :] - dp[:, DH:, :]).reshape(nh * DH, ts)


def _ds(i, size, align=None):
    if isinstance(i, int):
        return pl.ds(i * size, size)
    return pl.ds(pl.multiple_of(i * size, align or size), size)


def _rows(t):
    return _ds(t, TS)


def _kernel(x_hbm, wqkv_hbm, wphi_hbm, wo_hbm, w1_hbm, w2_hbm, dout_hbm,
            out_hbm, gx_hbm, dwqkv_hbm, dwphi_hbm, dwo_hbm, dw1_hbm, dw2_hbm,
            X, DO, WT, WOR, WPHI, BD, WO, W1, W2, XN, RSTD, PHIK, DQKV, R,
            DB, DS, OT, DXN, KVZ, DKVZ, DKVZB, DND, DHF, DWP, BB, PACC, DXA, DXB, PK0, FLAG,
            xsem, isem, osem):
    n_in = [0]

    def cin(src, dst):
        c = pltpu.make_async_copy(src, dst, isem.at[n_in[0]])
        n_in[0] += 1
        c.start()
        return c

    def x_copy(t):
        return pltpu.make_async_copy(x_hbm.at[_rows(t)], X.at[_rows(t)], xsem.at[t])

    def wrows(col, i):
        return cin(wqkv_hbm.at[pl.ds(512 * i, 512), pl.ds(col, D)],
                   WOR.at[pl.ds(512 * i, 512), pl.ds(col, D)])

    (O_OUT, O_GX, O_DWQKV, O_DWPHI, O_DWO, O_DW1, O_DW2) = range(7)

    def cout(src, dst, k):
        pltpu.make_async_copy(src, dst, osem.at[k]).start()

    FLAG[0] = 0
    x_copy(0).start()
    c_wk0 = wrows(D, 0)
    c_wphi = cin(wphi_hbm, WPHI)

    def bdmask():
        row = lax.broadcasted_iota(jnp.int32, (128, 128), 0)
        col = lax.broadcasted_iota(jnp.int32, (128, 128), 1)
        return (row // DH) == (col // DH)

    def emat():
        e_r = lax.broadcasted_iota(jnp.int32, (DH, 128), 0)
        e_c = lax.broadcasted_iota(jnp.int32, (DH, 128), 1)
        return jnp.where((e_c % DH) == e_r, 1.0, 0.0).astype(BF16)

    def m80():
        r80 = lax.broadcasted_iota(jnp.int32, (AUG, 128), 0)
        c80 = lax.broadcasted_iota(jnp.int32, (AUG, 128), 1)
        return jnp.where(r80 < 64, r80 // DH, (r80 - 64) // 8) == (c80 // 64)

    def ln_tile(t):
        rows = _rows(t)
        x = X[rows, :].astype(F32)
        mu = jnp.mean(x, axis=1, keepdims=True)
        xc = x - mu
        var = jnp.mean(xc * xc, axis=1, keepdims=True)
        rstd = lax.rsqrt(var + 1e-5)
        xn = (xc * rstd).astype(BF16)
        XN[rows, :] = xn
        RSTD[rows, :] = jnp.broadcast_to(rstd, (TS, 128))
        return xn

    def fold(g, off, rs=slice(None)):
        sl = pl.ds(off + g * 128, 128)
        WT[sl, rs] = _mm(BD[g], WOR[rs, sl], _TT).astype(BF16)

    def phik_tile(t, pk):
        rows = _rows(t)
        for c in range(8):
            PHIK[pl.ds(c * 256, 256), rows] = _softmax_pm(pk[c * 128:(c + 1) * 128]).astype(BF16)

    DKVZ[...] = jnp.zeros(DKVZ.shape, F32)
    PACC[...] = jnp.zeros(PACC.shape, F32)
    DXB[...] = jnp.zeros(DXB.shape, F32)
    DXN[...] = jnp.zeros(DXN.shape, F32)

    x_copy(0).wait()
    c_wk1 = wrows(D, 1)
    x_copy(1).start()
    xn0 = ln_tile(0)
    c_wphi.wait()
    c_wk0.wait()
    c_wv = cin(wqkv_hbm.at[:, pl.ds(2 * D, D)], WOR.at[:, pl.ds(2 * D, D)])
    for g in range(8):
        wrep = _mm(WPHI[pl.ds(g * 128, 128), :], emat(), _NN)
        BD[g] = jnp.where(bdmask(), wrep, 0.0).astype(BF16)
    for g in range(8):
        fold(g, D, pl.ds(0, 512))
    PK0[...] = _mm(WT[pl.ds(D, D), pl.ds(0, 512)], xn0[:, 0:512], _NT)
    c_wk1.wait()
    x_copy(1).wait()
    for t in range(2, NT):
        x_copy(t).start()
    for g in range(8):
        fold(g, D, pl.ds(512, 512))
    xn1 = ln_tile(1)
    phik_tile(0, PK0[...] + _mm(WT[pl.ds(D, D), pl.ds(512, 512)], xn0[:, 512:D], _NT))
    phik_tile(1, _mm(WT[pl.ds(D, D), :], xn1, _NT))
    c_wv.wait()
    x_copy(2).wait()
    wvt = WOR[:, pl.ds(2 * D, D)].T
    WT[pl.ds(2 * D, D), :] = wvt
    DQKV[pl.ds(2 * D, D), _rows(0)] = _mm(wvt, xn0, _NT).astype(BF16)
    DQKV[pl.ds(2 * D, D), _rows(1)] = _mm(wvt, xn1, _NT).astype(BF16)
    xn2 = ln_tile(2)
    DQKV[pl.ds(2 * D, D), _rows(2)] = _mm(wvt, xn2, _NT).astype(BF16)

    big = [(wqkv_hbm.at[:, pl.ds(0, D)], WOR.at[:, pl.ds(0, D)]), (w1_hbm, W1), (w2_hbm, W2),
           (dout_hbm, DO), (wo_hbm, WO)]
    nb = n_in[0]

    def big_copy(k):
        return pltpu.make_async_copy(big[k][0], big[k][1], isem.at[nb + k])

    def p1_step(t, xn):
        pk = _mm(WT[pl.ds(D, D), :], xn, _NT)
        xn_next = ln_tile(t + 1)
        vt = _mm(WT[pl.ds(2 * D, D), :], xn_next, _NT)
        phik_tile(t, pk)
        DQKV[pl.ds(2 * D, D), _rows(t + 1)] = vt.astype(BF16)
        return xn_next

    def p1_body(i, xn):
        x_copy(2 * i + 3).wait()
        x_copy(2 * i + 4).wait()

        @pl.when(i == 0)
        def _():
            for k in range(len(big)):
                big_copy(k).start()

        return p1_step(2 * i + 3, p1_step(2 * i + 2, xn))

    xn6 = lax.fori_loop(0, (NT - 4) // 2, p1_body, xn2)
    c_wq, c_w1, c_w2, c_do, c_wo = [big_copy(k) for k in range(len(big))]
    x_copy(NT - 1).wait()
    c_wq.wait()
    xn_last = p1_step(NT - 2, xn6)
    pk = _mm(WT[pl.ds(D, D), :], xn_last, _NT)
    for g in range(8):
        fold(g, 0)
    phik_tile(NT - 1, pk)

    c_w1.wait()

    def p1h_body(j, carry):
        fs = _ds(j, HC, 128)
        h = _mm(XN[...], W1[:, fs], _NN)
        R[:, fs] = jnp.where(h > 0.0, h, jnp.where(h == 0.0, 0.0, -0.0)).astype(BF16)
        return carry

    lax.fori_loop(0, NHC, p1h_body, 0)

    def ffn_b(t, c):
        cs = _ds(c, 256)
        BB[t % 2, :, cs] = _mm(R[_rows(t), :], W2[:, cs], _NN)

    ones_s = jnp.ones((16, S), BF16)
    for p in range(NP):
        v1 = jnp.concatenate([DQKV[pl.ds(2 * D + 64 * p, 64), :], ones_s], axis=0)
        kvz = _mm(v1, PHIK[pl.ds(128 * p, 128), :], _NT)
        KVZ[p] = jnp.where(m80(), kvz, 0.0).astype(BF16)

    c_w2.wait()

    def b0_body(c, carry):
        ffn_b(0, 2 * c)
        ffn_b(0, 2 * c + 1)
        return carry

    lax.fori_loop(0, 2, b0_body, 0)
    c_wo.wait()
    c_do.wait()

    def p2_tile(t, with_ffn):
        rows = _rows(t)
        b = BB[t % 2]
        sig = 0.5 * jnp.tanh(0.5 * b) + 0.5
        g = b * sig
        dout = DO[rows, :].astype(F32)
        ds = (dout * g).astype(BF16)
        e = dout * (sig + g * (1.0 - sig))
        DS[rows, :] = ds
        pq = _mm(WT[pl.ds(0, D), :], XN[rows, :], _NT)
        dot_ = _mm(WO[...], ds, _NT)
        if with_ffn:
            ffn_b(t + 1, 0)
        phiq = []
        for c in range(8):
            pc = _softmax_pm(pq[c * 128:(c + 1) * 128]).astype(BF16)
            phiq += [pc[0:128], pc[128:256]]
        nds = [_mm(KVZ[p], phiq[p], _NN) for p in range(NP)]
        if with_ffn:
            ffn_b(t + 1, 1)
        obs = []
        for p in range(NP):
            nd = nds[p]
            rden = _rcp(nd[64:AUG].reshape(2, 1, 8, TS) + 1e-6)
            o4 = nd[0:64].reshape(2, 4, 8, TS) * rden
            obs.append(o4.reshape(64, TS).astype(BF16))
            OT[pl.ds(64 * p, 64), rows] = obs[p]
            dnum = dot_[64 * p:64 * (p + 1)].reshape(2, 4, 8, TS) * rden
            dden = -jnp.sum(dnum * o4, axis=1, keepdims=True)
            DND[p, pl.ds(0, 64), :] = dnum.reshape(64, TS).astype(BF16)
            DND[p, pl.ds(64, 16), :] = dden.reshape(16, TS).astype(BF16)
        dphis = []
        for p in range(NP):
            dnd = DND[p]
            dphis.append(_mm(KVZ[p], dnd, _TN))
            DKVZ[p] += _mm(dnd, phiq[p], _NT)
        s = _mm(jnp.concatenate(obs, axis=0), WO[...], _TN)
        for p in range(NP):
            DQKV[pl.ds(64 * p, 64), rows] = _softmax_pm_bwd(phiq[p].astype(F32), dphis[p]).astype(BF16)
        if with_ffn:
            ffn_b(t + 1, 2)
            ffn_b(t + 1, 3)
        X[rows, :] = (X[rows, :].astype(F32) + s * g).astype(BF16)
        DB[rows, :] = (e * s).astype(BF16)

    def p2_body(t, carry):
        p2_tile(t, True)
        return carry

    lax.fori_loop(0, NT - 1, p2_body, 0)
    p2_tile(NT - 1, False)
    cout(X, out_hbm, O_OUT)

    for p in range(NP):
        DKVZB[p] = jnp.where(m80(), DKVZ[p], 0.0).astype(BF16)

    def kside(p):
        if isinstance(p, int):
            vs, ks = pl.ds(2 * D + 64 * p, 64), pl.ds(D + 64 * p, 64)
        else:
            vs = pl.ds(pl.multiple_of(2 * D + 64 * p, 64), 64)
            ks = pl.ds(pl.multiple_of(D + 64 * p, 64), 64)
        v1 = jnp.concatenate([DQKV[vs, :], ones_s], axis=0)
        dk = DKVZB[p]
        phi = PHIK[_ds(p, 128), :]
        dphi = _mm(dk, v1, _TN)
        DQKV[vs, :] = _mm(dk[0:64], phi, _NN).astype(BF16)
        DQKV[ks, :] = _softmax_pm_bwd(phi.astype(F32), dphi).astype(BF16)

    for p in range(NF, NP):
        kside(p)

    def p3_body(j, carry):
        fs = _ds(j, TF, 128)
        dr = _mm(DB[...], W2[fs, :], _NT)
        r = R[:, fs].astype(F32)
        rb = lax.bitcast_convert_type(r, jnp.int32)
        DHF[...] = jnp.where(r > 0.0, dr, jnp.where(rb == 0, 0.5 * dr, 0.0)).astype(BF16)
        W2[fs, :] = _mm(R[:, fs], DB[...], _TN).astype(BF16)
        cout(W2.at[fs, :], dw2_hbm.at[fs, :], O_DW2)
        kside(j)
        DXN[...] += _mm(DHF[...], W1[:, fs], _NT)
        W1[:, fs] = _mm(XN[...], DHF[...], _TN).astype(BF16)
        cout(W1.at[:, fs], dw1_hbm.at[:, fs], O_DW1)
        return carry

    lax.fori_loop(0, NF, p3_body, 0)

    def dwo_chunk(c):
        cs = _ds(c, 128)
        WO[:, cs] = _mm(OT[...], DS[:, cs], _NN).astype(BF16)

    def gx_tile(t, dx_ref, m1, m2):
        rows = _rows(t)
        xn = XN[rows, :].astype(F32)
        rstd = RSTD[rows, :][:, 0:1]
        return DO[rows, :].astype(F32) + rstd * (dx_ref[...] - m1 - xn * m2)

    pltpu.make_async_copy(X, out_hbm, osem.at[O_OUT]).wait()

    def p4_step(t, carry, prev_ref, cur_ref):
        never = FLAG[0] != 0
        rows = _rows(t)
        tp = jnp.maximum(t - 1, 0)
        dwo_chunk(t)
        dxn = _mm(DQKV[:, rows], WT[...], _TN) + DXN[rows, :]
        X[_rows(tp), :] = jnp.where(never, dxn, gx_tile(tp, prev_ref, *carry)).astype(BF16)
        m1 = jnp.mean(dxn, axis=1, keepdims=True)
        m2 = jnp.mean(dxn * XN[rows, :].astype(F32), axis=1, keepdims=True)
        cur_ref[...] = dxn
        return m1, m2

    def p4_body(i, carry):
        return p4_step(2 * i + 1, p4_step(2 * i, carry, DXB, DXA), DXA, DXB)

    zc = jnp.zeros((TS, 1), F32)
    m12 = lax.fori_loop(0, NT // 2, p4_body, (zc, zc))
    cout(WO, dwo_hbm, O_DWO)
    head = pl.ds(0, S - TS)
    cout(X.at[head], gx_hbm.at[head], O_GX)

    def p5_body(c, carry):
        cs = _ds(c, 512)
        gb = _mm(XN[...], DQKV[cs, :], _TT).astype(BF16)
        worig = WOR[:, cs]
        dws = []
        for gg in range(4):
            g = (c * 4 + gg) % 8
            gsl = gb[:, gg * 128:(gg + 1) * 128]
            PACC[g] += _mm(worig[:, gg * 128:(gg + 1) * 128], gsl, _TN)
            dws.append(_mm(gsl, BD[g], _NT).astype(BF16))
        WOR[:, cs] = jnp.concatenate(dws, axis=1)
        cout(WOR.at[:, cs], dwqkv_hbm.at[:, cs], O_DWQKV)
        return carry

    lax.fori_loop(0, 4, p5_body, 0)
    for g in range(8):
        pm = jnp.where(bdmask(), PACC[g], 0.0).astype(BF16)
        DWP[pl.ds(g * 128, 128), :] = _mm(pm, emat(), _NT).astype(BF16)
    cout(DWP, dwphi_hbm, O_DWPHI)
    off = 2 * D
    for w in (512, 256, 128, 128):
        cs = pl.ds(off, w)
        gv = _mm(XN[...], DQKV[cs, :], _TT)
        WOR[:, cs] = gv.astype(BF16)
        cout(WOR.at[:, cs], dwqkv_hbm.at[:, cs], O_DWQKV)
        if w == 512:
            anchor = jnp.concatenate([gv[0:TS], gv[2 * TS:3 * TS]], axis=1)
            X[_rows(NT - 1), :] = jnp.where(
                FLAG[0] != 0, anchor, gx_tile(NT - 1, DXB, *m12)).astype(BF16)
            cout(X.at[_rows(NT - 1)], gx_hbm.at[_rows(NT - 1)], O_GX)
        off += w

    for src, dst, k in ((W2, dw2_hbm, O_DW2), (W1, dw1_hbm, O_DW1), (WO, dwo_hbm, O_DWO),
                        (X, gx_hbm, O_GX), (DWP, dwphi_hbm, O_DWPHI), (WOR, dwqkv_hbm, O_DWQKV)):
        pltpu.make_async_copy(src, dst, osem.at[k]).wait()


@jax.jit
def pallas_recurrent_scan__linear_kernel_hedgehog__dense_activation_relu__prompt_kernel(
    A_x: jax.Array,
    A_wqkv: jax.Array,
    A_w_phi: jax.Array,
    A_wo: jax.Array,
    B_x: jax.Array,
    B_w1: jax.Array,
    B_w2: jax.Array,
    grad_out: jax.Array,
):
    x = A_x.reshape(S, D)
    dout = grad_out.reshape(S, D)
    wphi = A_w_phi.reshape(H * DH, DH)
    any_spec = pl.BlockSpec(memory_space=pl.ANY)
    out_shape = (
        jax.ShapeDtypeStruct((S, D), BF16),
        jax.ShapeDtypeStruct((S, D), BF16),
        jax.ShapeDtypeStruct((D, 3 * D), BF16),
        jax.ShapeDtypeStruct((H * DH, DH), BF16),
        jax.ShapeDtypeStruct((D, D), BF16),
        jax.ShapeDtypeStruct((D, FF), BF16),
        jax.ShapeDtypeStruct((FF, D), BF16),
    )
    scratch = [
        pltpu.VMEM((S, D), BF16),
        pltpu.VMEM((S, D), BF16),
        pltpu.VMEM((3 * D, D), BF16),
        pltpu.VMEM((D, 3 * D), BF16),
        pltpu.VMEM((H * DH, DH), BF16),
        pltpu.VMEM((8, 128, 128), BF16),
        pltpu.VMEM((D, D), BF16),
        pltpu.VMEM((D, FF), BF16),
        pltpu.VMEM((FF, D), BF16),
        pltpu.VMEM((S, D), BF16),
        pltpu.VMEM((S, 128), F32),
        pltpu.VMEM((2 * D, S), BF16),
        pltpu.VMEM((3 * D, S), BF16),
        pltpu.VMEM((S, FF), BF16),
        pltpu.VMEM((S, D), BF16),
        pltpu.VMEM((S, D), BF16),
        pltpu.VMEM((D, S), BF16),
        pltpu.VMEM((S, D), F32),
        pltpu.VMEM((NP, AUG, 128), BF16),
        pltpu.VMEM((NP, AUG, 128), F32),
        pltpu.VMEM((NP, AUG, 128), BF16),
        pltpu.VMEM((NP, AUG, TS), BF16),
        pltpu.VMEM((S, TF), BF16),
        pltpu.VMEM((H * DH, DH), BF16),
        pltpu.VMEM((2, TS, D), F32),
        pltpu.VMEM((8, 128, 128), F32),
        pltpu.VMEM((TS, D), F32),
        pltpu.VMEM((TS, D), F32),
        pltpu.VMEM((D, TS), F32),
        pltpu.SMEM((1,), jnp.int32),
        pltpu.SemaphoreType.DMA((NT,)),
        pltpu.SemaphoreType.DMA((16,)),
        pltpu.SemaphoreType.DMA((7,)),
    ]
    outs = pl.pallas_call(
        _kernel,
        in_specs=[any_spec] * 7,
        out_specs=[any_spec] * 7,
        out_shape=out_shape,
        scratch_shapes=scratch,
        compiler_params=pltpu.CompilerParams(vmem_limit_bytes=127 * 1024 * 1024),
    )(x, A_wqkv, wphi, A_wo, B_w1, B_w2, dout)
    out, gx, dwqkv, dwphi, dwo, dw1, dw2 = outs
    return (out.reshape(1, S, D), gx.reshape(1, S, D), dwqkv,
            dwphi.reshape(H, DH, DH), dwo, dw1, dw2)
```
